```python
import jax
import jax.numpy as jnp

def _softmax(x, axis=-1):
    return jax.nn.softmax(x, axis=axis)

def _gelu(x):
    return jax.nn.gelu(x, approximate=True)

def _silu(x):
    return jax.nn.silu(x)

def _sigmoid(x):
    return jax.nn.sigmoid(x)

def _layernorm(x, axis=-1, eps=1e-05):
    m = jnp.mean(x, axis=axis, keepdims=True)
    v = jnp.var(x, axis=axis, keepdims=True)
    return (x - m) / jnp.sqrt(v + eps)

def _scatter_add(tgt, idx, src, axis=0):
    return tgt.at[idx].add(src)

def _segment_sum(src, seg, n):
    return jax.ops.segment_sum(src, seg, n)

class _Rng:

    def __init__(self, key):
        self._k = key

    def _next(self):
        self._k, sub = jax.random.split(self._k)
        return sub

    def normal(self, shape):
        return jax.random.normal(self._next(), shape, dtype=jnp.bfloat16)

    def randint(self, lo, hi, shape):
        return jax.random.randint(self._next(), shape, lo, hi, dtype=jnp.int32)

    def uniform(self, shape, lo=0.0, hi=1.0):
        return jax.random.uniform(self._next(), shape, jnp.bfloat16, lo, hi)

    def permutation(self, n):
        return jax.random.permutation(self._next(), n)
kernel_name = 'adaLN_cond__sliding_block_cached__mixer_gmlp__decode'

def setup_inputs():
    _rng = _Rng(jax.random.key(int.from_bytes(__import__("os").urandom(4), "little")))
    _w = lambda a: (lambda t: t.astype(jnp.bfloat16) if jnp.issubdtype(t.dtype, jnp.floating) else t)(jnp.asarray(a))

    def _A_setup():
        B, Sq, D = (1, 1, 448)
        Hq, Hkv, Sk, Dh = (16, 8, 65536, 256)
        assert Hq % Hkv == 0, (Hq, Hkv)
        return {'x': _w((lambda *s: _rng.normal(s) * 0.05)(B, Sq, D)), 'k_cache': _w((lambda *s: _rng.normal(s) * 0.05)(B, Hkv, Sk, Dh)), 'v_cache': _w((lambda *s: _rng.normal(s) * 0.05)(B, Hkv, Sk, Dh)), 'wq': _w((lambda *s: _rng.normal(s) * 0.05)(D, Hq * Dh) * D ** (-0.5)), 'wo': _w((lambda *s: _rng.normal(s) * 0.05)(Hq * Dh, D) * (Hq * Dh) ** (-0.5))}
    _A_in = _A_setup()

    def _B_setup():
        B, S, D, F = (1, 1, 448, 1792)
        Fh = F // 2
        return {'x': _w((lambda *s: _rng.normal(s) * 0.05)(B, S, D)), 'w_in': _w((lambda *s: _rng.normal(s) * 0.05)(D, 2 * Fh)), 'w_sp': _w(0.01 * (lambda *s: _rng.normal(s) * 0.05)(S, S)), 'b_sp': _w(1.0 + 0.01 * (lambda *s: _rng.normal(s) * 0.05)(S)), 'w_out': _w((lambda *s: _rng.normal(s) * 0.05)(Fh, D))}
    _B_in = _B_setup()
    return {'A_x': _A_in['x'], 'A_k_cache': _A_in['k_cache'], 'A_v_cache': _A_in['v_cache'], 'A_wq': _A_in['wq'], 'A_wo': _A_in['wo'], 'B_x': _B_in['x'], 'B_w_in': _B_in['w_in'], 'B_w_sp': _B_in['w_sp'], 'B_b_sp': _B_in['b_sp'], 'B_w_out': _B_in['w_out'], 'c': _w((lambda *s: _rng.normal(s) * 0.05)(1, 448)), 'w_mod': _w((lambda *s: _rng.normal(s) * 0.05)(448, 6 * 448) * 448 ** (-0.5))}

def reference(A_x, A_k_cache, A_v_cache, A_wq, A_wo, B_x, B_w_in, B_w_sp, B_b_sp, B_w_out, c, w_mod):

    def _A_ref(x, k_cache, v_cache, wq, wo):
        B, Sq, D = x.shape
        Hq, Dh = (16, 256)
        Hkv, Sk = (k_cache.shape[1], k_cache.shape[2])
        W = min(4096, max(256, Sk // 4))
        rep = Hq // Hkv
        q = (lambda x, *d: x.transpose(*d))((x @ wq).reshape(B, Sq, Hq, Dh), 0, 2, 1, 3)
        k = jnp.repeat(k_cache[:, :, Sk - W:, :], rep, axis=1)
        v = jnp.repeat(v_cache[:, :, Sk - W:, :], rep, axis=1)
        scores = jnp.einsum('bhqd,bhkd->bhqk', q, k) * Dh ** (-0.5)
        p = _softmax(scores, axis=-1)
        o = jnp.einsum('bhqk,bhkd->bhqd', p, v)
        return (lambda x, *d: x.transpose(*d))(o, 0, 2, 1, 3).reshape(B, Sq, Hq * Dh) @ wo

    def _B_ref(x, w_in, w_sp, b_sp, w_out):
        B, S, D = x.shape
        F = w_in.shape[-1]
        Fh = F // 2
        z = _gelu(jnp.einsum('bsd,df->bsf', x, w_in))
        z1 = z[..., :Fh].copy()
        z2 = _layernorm(z[..., Fh:], axis=-1)
        g = jnp.einsum('ts,bsf->btf', w_sp, z2) + b_sp[None, :, None]
        return jnp.einsum('bsf,fd->bsd', z1 * g, w_out)
    x = A_x
    mod = (_silu(c) @ w_mod).reshape(c.shape[0], 6, 1, -1)
    sa, ca, ga, sb, cb, gb = (mod[:, 0].copy(), mod[:, 1].copy(), mod[:, 2].copy(), mod[:, 3].copy(), mod[:, 4].copy(), mod[:, 5].copy())
    h = _layernorm(x, axis=-1) * (1 + ca) + sa
    x = x + ga * _A_ref(h, A_k_cache, A_v_cache, A_wq, A_wo)
    h = _layernorm(x, axis=-1) * (1 + cb) + sb
    x = x + gb * _B_ref(h, B_w_in, B_w_sp, B_b_sp, B_w_out)
    return x
```

```python
import functools

import jax
import jax.numpy as jnp
from jax import lax
import jax.experimental.pallas as pl
import jax.experimental.pallas.tpu as pltpu

D = 448
HQ, HKV, DH = 16, 8, 256
FH = 896
EPS = 1e-5
BF16 = jnp.bfloat16
F32 = jnp.float32

_NT = (((1,), (1,)), ((), ()))
_NN = (((1,), (0,)), ((), ()))


def _ln(x):
    m = jnp.mean(x, axis=-1, keepdims=True)
    xc = x - m
    v = jnp.mean(xc * xc, axis=-1, keepdims=True)
    return xc * lax.rsqrt(v + EPS)


def _kernel(x_hbm, k_hbm, v_hbm, wq_hbm, woT_hbm, win_hbm, wsp_hbm, bsp_hbm, woutT_hbm, c_hbm, wmod_hbm,
            o_ref,
            xb, cb_, wspb, bspb, kbuf, vbuf, wq, woT, win, woutT, wmod, q_scr, o_scr, sems, *, SK, W):
    small = [
        pltpu.make_async_copy(c_hbm, cb_, sems.at[0]),
        pltpu.make_async_copy(x_hbm, xb, sems.at[1]),
        pltpu.make_async_copy(wsp_hbm, wspb, sems.at[2]),
        pltpu.make_async_copy(bsp_hbm, bspb, sems.at[3]),
    ]
    c_wmod = pltpu.make_async_copy(wmod_hbm, wmod, sems.at[4])
    c_wq = pltpu.make_async_copy(wq_hbm, wq, sems.at[5])
    c_wo = pltpu.make_async_copy(woT_hbm, woT, sems.at[6])
    c_win = pltpu.make_async_copy(win_hbm, win, sems.at[7])
    c_wout = pltpu.make_async_copy(woutT_hbm, woutT, sems.at[8])
    KB = 9
    VB = KB + HKV

    def k_copy(g):
        return pltpu.make_async_copy(k_hbm.at[0, g, pl.ds(SK - W, W), :], kbuf.at[g], sems.at[KB + g])

    def v_copy(g):
        return pltpu.make_async_copy(v_hbm.at[0, g, pl.ds(SK - W, W), :], vbuf.at[g], sems.at[VB + g])

    c_wmod.start()
    for cp in small:
        cp.start()
    c_wq.start()
    for g in range(HKV):
        k_copy(g).start()
        v_copy(g).start()
    c_wo.start()
    c_win.start()
    c_wout.start()

    for cp in small:
        cp.wait()
    c = jnp.broadcast_to(cb_[...].astype(F32), (8, D))
    x = jnp.broadcast_to(xb[0].astype(F32), (8, D))
    sc = (c * jax.nn.sigmoid(c)).astype(BF16)
    c_wmod.wait()
    mod = lax.dot_general(sc, wmod[...], _NN, preferred_element_type=F32)
    sa, ca, ga, sb, cb, gb = [mod[:, i * D:(i + 1) * D] for i in range(6)]
    h = (_ln(x) * (1.0 + ca) + sa).astype(BF16)
    c_wq.wait()
    q = lax.dot_general(h, wq[...], _NN, preferred_element_type=F32)
    q = (q.astype(BF16).astype(F32) * (DH ** -0.5))
    row_even = (lax.broadcasted_iota(jnp.int32, (8, DH), 0) % 2) == 0
    for g in range(HKV):
        qa = q[:, (2 * g) * DH:(2 * g + 1) * DH]
        qb = q[:, (2 * g + 1) * DH:(2 * g + 2) * DH]
        q_scr[g] = jnp.where(row_even, qa, qb)

    def head(g, carry):
        qg = q_scr[g].astype(BF16)
        k_copy(g).wait()
        s = lax.dot_general(qg, kbuf[g], _NT, preferred_element_type=F32)
        m = jnp.max(s, axis=-1, keepdims=True)
        e = jnp.exp(s - m)
        l = jnp.sum(e, axis=-1, keepdims=True)
        v_copy(g).wait()
        o = lax.dot_general(e.astype(BF16), vbuf[g], _NN, preferred_element_type=F32)
        o = o / l
        o_scr[g] = jnp.concatenate([jnp.where(row_even, o, 0.0), jnp.where(row_even, 0.0, o)], axis=1)
        return carry

    lax.fori_loop(0, HKV, head, 0)
    o_all = jnp.concatenate([o_scr[g] for g in range(HKV)], axis=1).astype(BF16)
    c_wo.wait()
    r = lax.dot_general(o_all, woT[...], _NT, preferred_element_type=F32)
    attn = r + pltpu.roll(r, 1, 0)
    x1 = x + ga * attn
    h2 = (_ln(x1) * (1.0 + cb) + sb).astype(BF16)
    c_win.wait()
    z = lax.dot_general(h2, win[...], _NN, preferred_element_type=F32)
    z = jax.nn.gelu(z, approximate=True)
    z1 = z[:, :FH]
    z2 = _ln(z[:, FH:])
    wsp = wspb[...].astype(F32)
    bsp = bspb[...].astype(F32).reshape(1, 1)
    gte = wsp * z2 + bsp
    zg = (z1 * gte).astype(BF16)
    c_wout.wait()
    y = lax.dot_general(zg, woutT[...], _NT, preferred_element_type=F32)
    x2 = x1 + gb * y
    o_ref[...] = x2[0:1, :].astype(BF16).reshape(1, 1, D)


@jax.jit
def pallas_adaLN_cond__sliding_block_cached__mixer_gmlp__decode_kernel(
    A_x: jax.Array,
    A_k_cache: jax.Array,
    A_v_cache: jax.Array,
    A_wq: jax.Array,
    A_wo: jax.Array,
    B_x: jax.Array,
    B_w_in: jax.Array,
    B_w_sp: jax.Array,
    B_b_sp: jax.Array,
    B_w_out: jax.Array,
    c: jax.Array,
    w_mod: jax.Array,
):
    del B_x
    SK = A_k_cache.shape[2]
    W = min(4096, max(256, SK // 4))
    hbm = pl.BlockSpec(memory_space=pltpu.HBM)
    return pl.pallas_call(
        functools.partial(_kernel, SK=SK, W=W),
        out_shape=jax.ShapeDtypeStruct((1, 1, D), BF16),
        in_specs=[hbm] * 11,
        out_specs=pl.BlockSpec(memory_space=pltpu.VMEM),
        scratch_shapes=[
            pltpu.VMEM((1, 1, D), BF16),
            pltpu.VMEM((1, D), BF16),
            pltpu.VMEM((1, 1), BF16),
            pltpu.VMEM((1,), BF16),
            pltpu.VMEM((HKV, W, DH), BF16),
            pltpu.VMEM((HKV, W, DH), BF16),
            pltpu.VMEM((D, HQ * DH), BF16),
            pltpu.VMEM((D, HQ * DH), BF16),
            pltpu.VMEM((D, 2 * FH), BF16),
            pltpu.VMEM((D, FH), BF16),
            pltpu.VMEM((D, 6 * D), BF16),
            pltpu.VMEM((HKV, 8, DH), F32),
            pltpu.VMEM((HKV, 8, 2 * DH), F32),
            pltpu.SemaphoreType.DMA((32,)),
        ],
        compiler_params=pltpu.CompilerParams(vmem_limit_bytes=100 * 1024 * 1024, disable_semaphore_checks=True),
    )(A_x, A_k_cache, A_v_cache, A_wq, A_wo.T, B_w_in, B_w_sp, B_b_sp, B_w_out.T, c, w_mod)
```

```python
import functools

import jax
import jax.numpy as jnp
from jax import lax
import jax.experimental.pallas as pl
import jax.experimental.pallas.tpu as pltpu

HQ, DH = 16, 256
EPS = 1e-5
BF16 = jnp.bfloat16
F32 = jnp.float32
ROWS = 8

_NN = (((1,), (0,)), ((), ()))
_NT = (((1,), (1,)), ((), ()))


def _dot(a, b, dims):
    return lax.dot_general(a, b, dims, preferred_element_type=F32)


def _layernorm(x):
    m = jnp.mean(x, axis=-1, keepdims=True)
    xc = x - m
    v = jnp.mean(xc * xc, axis=-1, keepdims=True)
    return xc * lax.rsqrt(v + EPS)


def _blocks(total, *cuts):
    edges = [0] + [c for c in cuts if 0 < c < total] + [total]
    return list(zip(edges[:-1], edges[1:]))


def _kernel(x_hbm, k_hbm, v_hbm, wq_hbm, wo_hbm, win_hbm, wsp_hbm, bsp_hbm, wout_hbm, c_hbm, wmod_hbm,
            out_ref,
            x_buf, c_buf, wsp_buf, bsp_buf, k_buf, v_buf, wq_buf, wo_buf, win_buf, wout_buf, wmod_buf,
            q_scr, o_scr, mod_scr, acc_scr, z_scr, sems, *, SK, W):
    HKV = k_buf.shape[0]
    D = wq_buf.shape[0]
    FH = wout_buf.shape[1]
    sem_ids = iter(range(sems.shape[0]))

    def copy(src, dst):
        return pltpu.make_async_copy(src, dst, sems.at[next(sem_ids)])

    def row_copies(src, dst, blocks):
        return [copy(src.at[pl.ds(lo, hi - lo), :], dst.at[pl.ds(lo, hi - lo), :]) for lo, hi in blocks]

    wo_blocks = _blocks(D, 128, 256, 384)
    win_blocks = _blocks(D, 256, 384)
    wout_blocks = _blocks(D, 128, 256, 384)

    small_cp = [copy(c_hbm, c_buf), copy(x_hbm, x_buf), copy(wsp_hbm, wsp_buf), copy(bsp_hbm, bsp_buf)]
    wmod_cp = copy(wmod_hbm, wmod_buf)
    wq_cp = copy(wq_hbm, wq_buf)
    wo_cp = row_copies(wo_hbm, wo_buf, wo_blocks)
    win_cp = row_copies(win_hbm, win_buf, win_blocks)
    wout_cp = row_copies(wout_hbm, wout_buf, wout_blocks)
    k_sem0 = next(sem_ids)
    v_sem0 = k_sem0 + HKV

    def k_cp(g):
        return pltpu.make_async_copy(k_hbm.at[0, g, pl.ds(SK - W, W), :], k_buf.at[g], sems.at[k_sem0 + g])

    def v_cp(g):
        return pltpu.make_async_copy(v_hbm.at[0, g, pl.ds(SK - W, W), :], v_buf.at[g], sems.at[v_sem0 + g])

    wmod_cp.start()
    for cp in small_cp:
        cp.start()
    wq_cp.start()
    for g in range(HKV):
        k_cp(g).start()
        v_cp(g).start()
    for cp in wo_cp + win_cp + wout_cp:
        cp.start()

    for cp in small_cp:
        cp.wait()
    c = jnp.broadcast_to(c_buf[...].astype(F32), (ROWS, D))
    x = jnp.broadcast_to(x_buf[0].astype(F32), (ROWS, D))
    silu_c = (c * jax.nn.sigmoid(c)).astype(BF16)
    wmod_cp.wait()
    mod = _dot(silu_c, wmod_buf[...], _NN)
    for i in range(6):
        mod_scr[i] = mod[:, i * D:(i + 1) * D]

    h = (_layernorm(x) * (1.0 + mod_scr[1]) + mod_scr[0]).astype(BF16)
    wq_cp.wait()
    q = _dot(h, wq_buf[...], _NN)
    q = q.astype(BF16).astype(F32) * (DH ** -0.5)
    even = (lax.broadcasted_iota(jnp.int32, (ROWS, DH), 0) % 2) == 0
    for g in range(HKV):
        q_scr[g] = jnp.where(even, q[:, (2 * g) * DH:(2 * g + 1) * DH], q[:, (2 * g + 1) * DH:(2 * g + 2) * DH])

    def kv_head(g, carry):
        qg = q_scr[g].astype(BF16)
        k_cp(g).wait()
        s = _dot(qg, k_buf[g], _NT)
        e = jnp.exp(s - jnp.max(s, axis=-1, keepdims=True))
        denom = jnp.sum(e, axis=-1, keepdims=True)
        v_cp(g).wait()
        o = _dot(e.astype(BF16), v_buf[g], _NN) / denom
        o_scr[g] = jnp.concatenate([jnp.where(even, o, 0.0), jnp.where(even, 0.0, o)], axis=1)
        return carry

    lax.fori_loop(0, HKV, kv_head, 0)

    o_all = jnp.concatenate([o_scr[g] for g in range(HKV)], axis=1).astype(BF16)
    for cp, (lo, hi) in zip(wo_cp, wo_blocks):
        cp.wait()
        acc_scr[0, :, lo:hi] = _dot(o_all, wo_buf[lo:hi, :], _NT)
    r = acc_scr[0]
    x1 = x + mod_scr[2] * (r + pltpu.roll(r, 1, 0))

    h2 = (_layernorm(x1) * (1.0 + mod_scr[4]) + mod_scr[3]).astype(BF16)
    for i, (cp, (lo, hi)) in enumerate(zip(win_cp, win_blocks)):
        cp.wait()
        part = _dot(h2[:, lo:hi], win_buf[lo:hi, :], _NN)
        if i == len(win_blocks) - 1:
            z = z_scr[...] + part
        elif i == 0:
            z_scr[...] = part
        else:
            z_scr[...] += part
    z = jax.nn.gelu(z, approximate=True)
    w_sp = wsp_buf[...].astype(F32)
    b_sp = bsp_buf[...].astype(F32).reshape(1, 1)
    gate = w_sp * _layernorm(z[:, FH:]) + b_sp
    zg = (z[:, :FH] * gate).astype(BF16)

    last_lo = wout_blocks[-1][0]
    for cp, (lo, hi) in zip(wout_cp, wout_blocks):
        cp.wait()
        y = _dot(zg, wout_buf[lo:hi, :], _NT)
        if lo != last_lo:
            acc_scr[1, :, lo:hi] = y
    x2 = jnp.concatenate([x1[:, :last_lo] + mod_scr[5, :, :last_lo] * acc_scr[1, :, :last_lo],
                          x1[:, last_lo:] + mod_scr[5, :, last_lo:] * y], axis=1)
    out_ref[...] = x2[0:1, :].astype(BF16).reshape(out_ref.shape)


@jax.jit
def pallas_adaLN_cond__sliding_block_cached__mixer_gmlp__decode_kernel(
    A_x: jax.Array,
    A_k_cache: jax.Array,
    A_v_cache: jax.Array,
    A_wq: jax.Array,
    A_wo: jax.Array,
    B_x: jax.Array,
    B_w_in: jax.Array,
    B_w_sp: jax.Array,
    B_b_sp: jax.Array,
    B_w_out: jax.Array,
    c: jax.Array,
    w_mod: jax.Array,
):
    del B_x
    D = A_x.shape[-1]
    HKV, SK = A_k_cache.shape[1], A_k_cache.shape[2]
    W = min(4096, max(256, SK // 4))
    FH = B_w_out.shape[0]
    n_sems = 6 + 4 + 3 + 4 + 2 * HKV
    hbm = pl.BlockSpec(memory_space=pltpu.HBM)
    return pl.pallas_call(
        functools.partial(_kernel, SK=SK, W=W),
        out_shape=jax.ShapeDtypeStruct(A_x.shape, BF16),
        in_specs=[hbm] * 11,
        out_specs=pl.BlockSpec(memory_space=pltpu.VMEM),
        scratch_shapes=[
            pltpu.VMEM(A_x.shape, BF16),
            pltpu.VMEM(c.shape, BF16),
            pltpu.VMEM(B_w_sp.shape, BF16),
            pltpu.VMEM(B_b_sp.shape, BF16),
            pltpu.VMEM((HKV, W, DH), BF16),
            pltpu.VMEM((HKV, W, DH), BF16),
            pltpu.VMEM((D, HQ * DH), BF16),
            pltpu.VMEM((D, HQ * DH), BF16),
            pltpu.VMEM((D, 2 * FH), BF16),
            pltpu.VMEM((D, FH), BF16),
            pltpu.VMEM((D, 6 * D), BF16),
            pltpu.VMEM((HKV, ROWS, DH), F32),
            pltpu.VMEM((HKV, ROWS, 2 * DH), F32),
            pltpu.VMEM((6, ROWS, D), F32),
            pltpu.VMEM((2, ROWS, D), F32),
            pltpu.VMEM((ROWS, 2 * FH), F32),
            pltpu.SemaphoreType.DMA((n_sems,)),
        ],
        compiler_params=pltpu.CompilerParams(
            vmem_limit_bytes=100 * 1024 * 1024,
            disable_semaphore_checks=True,
        ),
    )(A_x, A_k_cache, A_v_cache, A_wq, A_wo.T, B_w_in, B_w_sp, B_b_sp, B_w_out.T, c, w_mod)
```

```python
import functools

import jax
import jax.numpy as jnp
from jax import lax
import jax.experimental.pallas as pl
import jax.experimental.pallas.tpu as pltpu

HQ, DH = 16, 256
EPS = 1e-5
BF16 = jnp.bfloat16
F32 = jnp.float32
ROWS = 8
KV_PIECE_ROWS = 160
LOOKAHEAD = 3

_NN = (((1,), (0,)), ((), ()))
_NT = (((1,), (1,)), ((), ()))


def _dot(a, b, dims):
    return lax.dot_general(a, b, dims, preferred_element_type=F32)


def _layernorm(x):
    m = jnp.mean(x, axis=-1, keepdims=True)
    xc = x - m
    v = jnp.mean(xc * xc, axis=-1, keepdims=True)
    return xc * lax.rsqrt(v + EPS)


def _blocks(total, *cuts):
    edges = [0] + [c for c in cuts if 0 < c < total] + [total]
    return list(zip(edges[:-1], edges[1:]))


def _steps(total, step):
    return _blocks(total, *range(step, total, step))


def _kernel(x_hbm, k_hbm, v_hbm, wq_hbm, wo_hbm, win_hbm, wsp_hbm, bsp_hbm, wout_hbm, c_hbm, wmod_hbm,
            out_ref,
            x_buf, c_buf, wsp_buf, bsp_buf, k_buf, v_buf, wq_buf, wo_buf, win_buf, wout_buf, wmod_buf,
            q_scr, o_scr, mod_scr, acc_scr, z_scr, sems, *, SK, W):
    HKV = k_buf.shape[0]
    D = wq_buf.shape[0]
    FH = wout_buf.shape[1]
    look = min(LOOKAHEAD, HKV)

    wo_blocks = _blocks(D, 128, 256, 384)
    win_blocks = _blocks(D, 256, 384)
    wout_blocks = _blocks(D, 128, 256, 384)

    S_SMALL, S_WMOD, S_WQ, S_K = 0, 4, 5, 6
    S_V = S_K + HKV
    S_WO = S_V + HKV
    S_WIN = S_WO + len(wo_blocks)
    S_WOUT = S_WIN + len(win_blocks)

    def start_rows(src, dst, blocks, sem_id, priority):
        for i, (lo, hi) in enumerate(blocks):
            pltpu.make_async_copy(
                src.at[pl.ds(lo, hi - lo), :], dst.at[pl.ds(lo, hi - lo), :], sems.at[sem_id]
            ).start(priority=i % 2 if priority is None else priority)

    def wait_filled(buf, sem_id):
        pltpu.make_async_copy(buf, buf, sems.at[sem_id]).wait()

    kv_pieces = _steps(W, KV_PIECE_ROWS)

    def start_k(g):
        start_rows(k_hbm.at[0, g, pl.ds(SK - W, W), :], k_buf.at[g], kv_pieces, S_K + g, None)

    def start_v(g):
        start_rows(v_hbm.at[0, g, pl.ds(SK - W, W), :], v_buf.at[g], kv_pieces, S_V + g, None)

    small = ((c_hbm, c_buf), (x_hbm, x_buf), (wsp_hbm, wsp_buf), (bsp_hbm, bsp_buf))
    for i, (src, dst) in enumerate(small):
        pltpu.make_async_copy(src, dst, sems.at[S_SMALL + i]).start(priority=0)
    start_rows(wmod_hbm, wmod_buf, _steps(D, 16), S_WMOD, 1)
    start_rows(wq_hbm, wq_buf, _steps(D, 8), S_WQ, 1)
    first_kv = [functools.partial(f, g) for g in range(look) for f in (start_k, start_v)]
    for start in first_kv[:3]:
        start()

    for i, (_, dst) in enumerate(small):
        wait_filled(dst, S_SMALL + i)
    c = jnp.broadcast_to(c_buf[...].astype(F32), (ROWS, D))
    x = jnp.broadcast_to(x_buf[0].astype(F32), (ROWS, D))
    silu_c = (c * jax.nn.sigmoid(c)).astype(BF16)
    wait_filled(wmod_buf, S_WMOD)
    mod = _dot(silu_c, wmod_buf[...], _NN)
    for i in range(6):
        mod_scr[i] = mod[:, i * D:(i + 1) * D]

    h = (_layernorm(x) * (1.0 + mod_scr[1]) + mod_scr[0]).astype(BF16)
    for start in first_kv[3:]:
        start()
    wait_filled(wq_buf, S_WQ)
    q = _dot(h, wq_buf[...], _NN)
    q = q.astype(BF16).astype(F32) * (DH ** -0.5)
    even = (lax.broadcasted_iota(jnp.int32, (ROWS, DH), 0) % 2) == 0
    for g in range(HKV):
        q_scr[g] = jnp.where(even, q[:, (2 * g) * DH:(2 * g + 1) * DH], q[:, (2 * g + 1) * DH:(2 * g + 2) * DH])

    def kv_head(g, carry, *, prefetch):
        qg = q_scr[g].astype(BF16)
        if prefetch:
            start_k(g + look)
        wait_filled(k_buf.at[g], S_K + g)
        s = _dot(qg, k_buf[g], _NT)
        e = jnp.exp(s - jnp.max(s, axis=-1, keepdims=True))
        denom = jnp.sum(e, axis=-1, keepdims=True)
        if prefetch:
            start_v(g + look)
        wait_filled(v_buf.at[g], S_V + g)
        o = _dot(e.astype(BF16), v_buf[g], _NN) / denom
        o_scr[g] = jnp.concatenate([jnp.where(even, o, 0.0), jnp.where(even, 0.0, o)], axis=1)
        return carry

    lax.fori_loop(0, HKV - look, functools.partial(kv_head, prefetch=True), 0)
    for i, blk in enumerate(wo_blocks):
        start_rows(wo_hbm, wo_buf, [blk], S_WO + i, 1)
    for i, blk in enumerate(win_blocks):
        start_rows(win_hbm, win_buf, [blk], S_WIN + i, 1)
    for i, blk in enumerate(wout_blocks):
        start_rows(wout_hbm, wout_buf, [blk], S_WOUT + i, 1)
    lax.fori_loop(HKV - look, HKV, functools.partial(kv_head, prefetch=False), 0)

    o_all = jnp.concatenate([o_scr[g] for g in range(HKV)], axis=1).astype(BF16)
    for i, (lo, hi) in enumerate(wo_blocks):
        wait_filled(wo_buf.at[pl.ds(lo, hi - lo), :], S_WO + i)
        acc_scr[0, :, lo:hi] = _dot(o_all, wo_buf[lo:hi, :], _NT)
    r = acc_scr[0]
    x1 = x + mod_scr[2] * (r + pltpu.roll(r, 1, 0))

    h2 = (_layernorm(x1) * (1.0 + mod_scr[4]) + mod_scr[3]).astype(BF16)
    for i, (lo, hi) in enumerate(win_blocks):
        wait_filled(win_buf.at[pl.ds(lo, hi - lo), :], S_WIN + i)
        part = _dot(h2[:, lo:hi], win_buf[lo:hi, :], _NN)
        if i == len(win_blocks) - 1:
            z = z_scr[...] + part
        elif i == 0:
            z_scr[...] = part
        else:
            z_scr[...] += part
    z = jax.nn.gelu(z, approximate=True)
    w_sp = wsp_buf[...].astype(F32)
    b_sp = bsp_buf[...].astype(F32).reshape(1, 1)
    gate = w_sp * _layernorm(z[:, FH:]) + b_sp
    zg = (z[:, :FH] * gate).astype(BF16)

    last_lo = wout_blocks[-1][0]
    for i, (lo, hi) in enumerate(wout_blocks):
        wait_filled(wout_buf.at[pl.ds(lo, hi - lo), :], S_WOUT + i)
        y = _dot(zg, wout_buf[lo:hi, :], _NT)
        if lo != last_lo:
            acc_scr[1, :, lo:hi] = y
    x2 = jnp.concatenate([x1[:, :last_lo] + mod_scr[5, :, :last_lo] * acc_scr[1, :, :last_lo],
                          x1[:, last_lo:] + mod_scr[5, :, last_lo:] * y], axis=1)
    out_ref[...] = x2[0:1, :].astype(BF16).reshape(out_ref.shape)


@jax.jit
def pallas_adaLN_cond__sliding_block_cached__mixer_gmlp__decode_kernel(
    A_x: jax.Array,
    A_k_cache: jax.Array,
    A_v_cache: jax.Array,
    A_wq: jax.Array,
    A_wo: jax.Array,
    B_x: jax.Array,
    B_w_in: jax.Array,
    B_w_sp: jax.Array,
    B_b_sp: jax.Array,
    B_w_out: jax.Array,
    c: jax.Array,
    w_mod: jax.Array,
):
    del B_x
    D = A_x.shape[-1]
    HKV, SK = A_k_cache.shape[1], A_k_cache.shape[2]
    W = min(4096, max(256, SK // 4))
    FH = B_w_out.shape[0]
    n_sems = 6 + 2 * HKV + 4 + 3 + 4
    hbm = pl.BlockSpec(memory_space=pltpu.HBM)
    return pl.pallas_call(
        functools.partial(_kernel, SK=SK, W=W),
        out_shape=jax.ShapeDtypeStruct(A_x.shape, BF16),
        in_specs=[hbm] * 11,
        out_specs=pl.BlockSpec(memory_space=pltpu.VMEM),
        scratch_shapes=[
            pltpu.VMEM(A_x.shape, BF16),
            pltpu.VMEM(c.shape, BF16),
            pltpu.VMEM(B_w_sp.shape, BF16),
            pltpu.VMEM(B_b_sp.shape, BF16),
            pltpu.VMEM((HKV, W, DH), BF16),
            pltpu.VMEM((HKV, W, DH), BF16),
            pltpu.VMEM((D, HQ * DH), BF16),
            pltpu.VMEM((D, HQ * DH), BF16),
            pltpu.VMEM((D, 2 * FH), BF16),
            pltpu.VMEM((D, FH), BF16),
            pltpu.VMEM((D, 6 * D), BF16),
            pltpu.VMEM((HKV, ROWS, DH), F32),
            pltpu.VMEM((HKV, ROWS, 2 * DH), F32),
            pltpu.VMEM((6, ROWS, D), F32),
            pltpu.VMEM((2, ROWS, D), F32),
            pltpu.VMEM((ROWS, 2 * FH), F32),
            pltpu.SemaphoreType.DMA((n_sems,)),
        ],
        compiler_params=pltpu.CompilerParams(
            vmem_limit_bytes=100 * 1024 * 1024,
            disable_semaphore_checks=True,
        ),
    )(A_x, A_k_cache, A_v_cache, A_wq, A_wo.T, B_w_in, B_w_sp, B_b_sp, B_w_out.T, c, w_mod)
```

```python
import functools

import jax
import jax.numpy as jnp
from jax import lax
import jax.experimental.pallas as pl
import jax.experimental.pallas.tpu as pltpu

HQ, DH = 16, 256
EPS = 1e-5
BF16 = jnp.bfloat16
F32 = jnp.float32
ROWS = 8
LOOKAHEAD = 3
KV_CYCLE = ((160, 0), (96, 1))
K_PHASE, V_PHASE = 96, 128

_NN = (((1,), (0,)), ((), ()))
_NT = (((1,), (1,)), ((), ()))


def _dot(a, b, dims):
    return lax.dot_general(a, b, dims, preferred_element_type=F32)


def _layernorm(x):
    m = jnp.mean(x, axis=-1, keepdims=True)
    xc = x - m
    v = jnp.mean(xc * xc, axis=-1, keepdims=True)
    return xc * lax.rsqrt(v + EPS)


def _blocks(total, *cuts):
    edges = [0] + [c for c in cuts if 0 < c < total] + [total]
    return list(zip(edges[:-1], edges[1:]))


def _steps(total, step, priority):
    return [(lo, hi, i % 2 if priority is None else priority)
            for i, (lo, hi) in enumerate(_blocks(total, *range(step, total, step)))]


def _cycle(total, cycle, phase):
    out, lo, i = [], 0, 0
    while phase >= cycle[i][0]:
        phase -= cycle[i][0]
        i = (i + 1) % len(cycle)
    while lo < total:
        rows, priority = cycle[i]
        hi = min(lo + rows - phase, total)
        out.append((lo, hi, priority))
        lo, phase, i = hi, 0, (i + 1) % len(cycle)
    return out


def _kernel(x_hbm, k_hbm, v_hbm, wq_hbm, wo_hbm, win_hbm, wsp_hbm, bsp_hbm, wout_hbm, c_hbm, wmod_hbm,
            out_ref,
            x_buf, c_buf, wsp_buf, bsp_buf, k_buf, v_buf, wq_buf, wo_buf, win_buf, wout_buf, wmod_buf,
            q_scr, o_scr, mod_scr, acc_scr, z_scr, sems, *, SK, W):
    HKV = k_buf.shape[0]
    D = wq_buf.shape[0]
    FH = wout_buf.shape[1]
    look = min(LOOKAHEAD, HKV)

    wo_blocks = _blocks(D, 384)
    win_blocks = _blocks(D, 256, 384)
    wout_blocks = _blocks(D, 128, 256, 384)

    S_SMALL, S_WMOD, S_WQ, S_K = 0, 4, 5, 6
    S_V = S_K + HKV
    S_WO = S_V + HKV
    S_WIN = S_WO + len(wo_blocks)
    S_WOUT = S_WIN + len(win_blocks)

    def start_rows(src, dst, pieces, sem_id):
        for lo, hi, priority in pieces:
            pltpu.make_async_copy(
                src.at[pl.ds(lo, hi - lo), :], dst.at[pl.ds(lo, hi - lo), :], sems.at[sem_id]
            ).start(priority=priority)

    def wait_filled(buf, sem_id):
        pltpu.make_async_copy(buf, buf, sems.at[sem_id]).wait()

    k_pieces = _cycle(W, KV_CYCLE, K_PHASE)
    v_pieces = _cycle(W, KV_CYCLE, V_PHASE)

    def start_k(g):
        start_rows(k_hbm.at[0, g, pl.ds(SK - W, W), :], k_buf.at[g], k_pieces, S_K + g)

    def start_v(g):
        start_rows(v_hbm.at[0, g, pl.ds(SK - W, W), :], v_buf.at[g], v_pieces, S_V + g)

    def start_wo_head():
        start_rows(wo_hbm, wo_buf, _steps(wo_blocks[0][1], 8, None), S_WO)

    small = ((c_hbm, c_buf), (x_hbm, x_buf), (wsp_hbm, wsp_buf), (bsp_hbm, bsp_buf))
    for i, (src, dst) in enumerate(small):
        pltpu.make_async_copy(src, dst, sems.at[S_SMALL + i]).start(priority=0)
    start_rows(wmod_hbm, wmod_buf, _steps(D, 16, 1), S_WMOD)
    start_rows(wq_hbm, wq_buf, _steps(D, 8, 1), S_WQ)
    first = [functools.partial(f, g) for g in range(look) for f in (start_k, start_v)]
    first.insert(2, start_wo_head)
    for start in first[:3]:
        start()

    for i, (_, dst) in enumerate(small):
        wait_filled(dst, S_SMALL + i)
    c = jnp.broadcast_to(c_buf[...].astype(F32), (ROWS, D))
    x = jnp.broadcast_to(x_buf[0].astype(F32), (ROWS, D))
    silu_c = (c * jax.nn.sigmoid(c)).astype(BF16)
    wait_filled(wmod_buf, S_WMOD)
    mod = _dot(silu_c, wmod_buf[...], _NN)
    for i in range(6):
        mod_scr[i] = mod[:, i * D:(i + 1) * D]

    h = (_layernorm(x) * (1.0 + mod_scr[1]) + mod_scr[0]).astype(BF16)
    for start in first[3:]:
        start()
    wait_filled(wq_buf, S_WQ)
    q = _dot(h, wq_buf[...], _NN)
    q = q.astype(BF16).astype(F32) * (DH ** -0.5)
    even = (lax.broadcasted_iota(jnp.int32, (ROWS, DH), 0) % 2) == 0
    for g in range(HKV):
        q_scr[g] = jnp.where(even, q[:, (2 * g) * DH:(2 * g + 1) * DH], q[:, (2 * g + 1) * DH:(2 * g + 2) * DH])

    def kv_head(g, carry, *, prefetch):
        qg = q_scr[g].astype(BF16)
        if prefetch:
            start_k(g + look)
        wait_filled(k_buf.at[g], S_K + g)
        s = _dot(qg, k_buf[g], _NT)
        e = jnp.exp(s - jnp.max(s, axis=-1, keepdims=True))
        denom = jnp.sum(e, axis=-1, keepdims=True)
        if prefetch:
            start_v(g + look)
        wait_filled(v_buf.at[g], S_V + g)
        o = _dot(e.astype(BF16), v_buf[g], _NN) / denom
        o_scr[g] = jnp.concatenate([jnp.where(even, o, 0.0), jnp.where(even, 0.0, o)], axis=1)
        return carry

    lax.fori_loop(0, HKV - look, functools.partial(kv_head, prefetch=True), 0)
    for i, (lo, hi) in enumerate(wo_blocks[1:], 1):
        start_rows(wo_hbm, wo_buf, [(lo, hi, 1)], S_WO + i)
    for i, (lo, hi) in enumerate(win_blocks):
        start_rows(win_hbm, win_buf, [(lo, hi, 1)], S_WIN + i)
    for i, (lo, hi) in enumerate(wout_blocks):
        start_rows(wout_hbm, wout_buf, [(lo, hi, 1)], S_WOUT + i)
    lax.fori_loop(HKV - look, HKV, functools.partial(kv_head, prefetch=False), 0)

    o_all = jnp.concatenate([o_scr[g] for g in range(HKV)], axis=1).astype(BF16)
    for i, (lo, hi) in enumerate(wo_blocks):
        wait_filled(wo_buf.at[pl.ds(lo, hi - lo), :], S_WO + i)
        acc_scr[0, :, lo:hi] = _dot(o_all, wo_buf[lo:hi, :], _NT)
    r = acc_scr[0]
    x1 = x + mod_scr[2] * (r + pltpu.roll(r, 1, 0))

    h2 = (_layernorm(x1) * (1.0 + mod_scr[4]) + mod_scr[3]).astype(BF16)
    for i, (lo, hi) in enumerate(win_blocks):
        wait_filled(win_buf.at[pl.ds(lo, hi - lo), :], S_WIN + i)
        part = _dot(h2[:, lo:hi], win_buf[lo:hi, :], _NN)
        if i == len(win_blocks) - 1:
            z = z_scr[...] + part
        elif i == 0:
            z_scr[...] = part
        else:
            z_scr[...] += part
    z = jax.nn.gelu(z, approximate=True)
    w_sp = wsp_buf[...].astype(F32)
    b_sp = bsp_buf[...].astype(F32).reshape(1, 1)
    gate = w_sp * _layernorm(z[:, FH:]) + b_sp
    zg = (z[:, :FH] * gate).astype(BF16)

    last_lo = wout_blocks[-1][0]
    for i, (lo, hi) in enumerate(wout_blocks):
        wait_filled(wout_buf.at[pl.ds(lo, hi - lo), :], S_WOUT + i)
        y = _dot(zg, wout_buf[lo:hi, :], _NT)
        if lo != last_lo:
            acc_scr[1, :, lo:hi] = y
    x2 = jnp.concatenate([x1[:, :last_lo] + mod_scr[5, :, :last_lo] * acc_scr[1, :, :last_lo],
                          x1[:, last_lo:] + mod_scr[5, :, last_lo:] * y], axis=1)
    out_ref[...] = x2[0:1, :].astype(BF16).reshape(out_ref.shape)


@jax.jit
def pallas_adaLN_cond__sliding_block_cached__mixer_gmlp__decode_kernel(
    A_x: jax.Array,
    A_k_cache: jax.Array,
    A_v_cache: jax.Array,
    A_wq: jax.Array,
    A_wo: jax.Array,
    B_x: jax.Array,
    B_w_in: jax.Array,
    B_w_sp: jax.Array,
    B_b_sp: jax.Array,
    B_w_out: jax.Array,
    c: jax.Array,
    w_mod: jax.Array,
):
    del B_x
    D = A_x.shape[-1]
    HKV, SK = A_k_cache.shape[1], A_k_cache.shape[2]
    W = min(4096, max(256, SK // 4))
    FH = B_w_out.shape[0]
    n_sems = 6 + 2 * HKV + 2 + 3 + 4
    hbm = pl.BlockSpec(memory_space=pltpu.HBM)
    return pl.pallas_call(
        functools.partial(_kernel, SK=SK, W=W),
        out_shape=jax.ShapeDtypeStruct(A_x.shape, BF16),
        in_specs=[hbm] * 11,
        out_specs=pl.BlockSpec(memory_space=pltpu.VMEM),
        scratch_shapes=[
            pltpu.VMEM(A_x.shape, BF16),
            pltpu.VMEM(c.shape, BF16),
            pltpu.VMEM(B_w_sp.shape, BF16),
            pltpu.VMEM(B_b_sp.shape, BF16),
            pltpu.VMEM((HKV, W, DH), BF16),
            pltpu.VMEM((HKV, W, DH), BF16),
            pltpu.VMEM((D, HQ * DH), BF16),
            pltpu.VMEM((D, HQ * DH), BF16),
            pltpu.VMEM((D, 2 * FH), BF16),
            pltpu.VMEM((D, FH), BF16),
            pltpu.VMEM((D, 6 * D), BF16),
            pltpu.VMEM((HKV, ROWS, DH), F32),
            pltpu.VMEM((HKV, ROWS, 2 * DH), F32),
            pltpu.VMEM((6, ROWS, D), F32),
            pltpu.VMEM((2, ROWS, D), F32),
            pltpu.VMEM((ROWS, 2 * FH), F32),
            pltpu.SemaphoreType.DMA((n_sems,)),
        ],
        compiler_params=pltpu.CompilerParams(
            vmem_limit_bytes=100 * 1024 * 1024,
            disable_semaphore_checks=True,
        ),
    )(A_x, A_k_cache, A_v_cache, A_wq, A_wo.T, B_w_in, B_w_sp, B_b_sp, B_w_out.T, c, w_mod)
```

```python
import functools

import jax
import jax.numpy as jnp
from jax import lax
import jax.experimental.pallas as pl
import jax.experimental.pallas.tpu as pltpu

HQ, DH = 16, 256
EPS = 1e-5
BF16 = jnp.bfloat16
F32 = jnp.float32
ROWS = 8

TILE_R, TILE_C = 8, 128
CYCLE = (40, 24)
K_PHASE, V_PHASE = 24, 32
LEAD = 32
LOOKAHEAD = 2

_NN = (((1,), (0,)), ((), ()))
_NT = (((1,), (1,)), ((), ()))


def _dot(a, b, dims):
    return lax.dot_general(a, b, dims, preferred_element_type=F32)


def _layernorm(x):
    m = jnp.mean(x, axis=-1, keepdims=True)
    xc = x - m
    v = jnp.mean(xc * xc, axis=-1, keepdims=True)
    return xc * lax.rsqrt(v + EPS)


def _blocks(total, *cuts):
    edges = [0] + [c for c in cuts if 0 < c < total] + [total]
    return list(zip(edges[:-1], edges[1:]))


def _rects(t0, t1, col_tiles):
    out = []
    while t0 < t1:
        r, c = divmod(t0, col_tiles)
        if c == 0 and t1 - t0 >= col_tiles:
            n = (t1 - t0) // col_tiles
            out.append((r * TILE_R, n * TILE_R, 0, col_tiles * TILE_C))
            t0 += n * col_tiles
        else:
            n = min(col_tiles - c, t1 - t0)
            out.append((r * TILE_R, TILE_R, c * TILE_C, n * TILE_C))
            t0 += n
    return out


def _two_queues(shape, lo, hi, phase=0):
    col_tiles = shape[1] // TILE_C
    t, end = lo // TILE_R * col_tiles, hi // TILE_R * col_tiles
    queues, held = ([], []), []
    pos = (t + phase) % sum(CYCLE)
    while t < end:
        prio = 0 if pos < CYCLE[0] else 1
        n = min((CYCLE[0] if prio == 0 else sum(CYCLE)) - pos, end - t)
        piece = _rects(t, t + n, col_tiles)
        if prio == 0 and not queues[1] and n < CYCLE[0] and not held:
            held = piece
        else:
            queues[prio].append(held + piece if prio == 0 else piece)
            held = [] if prio == 0 else held
        t, pos = t + n, (pos + n) % sum(CYCLE)
    if held:
        queues[0].append(held)
    return queues


def _kernel(x_hbm, k_hbm, v_hbm, wq_hbm, wo_hbm, win_hbm, wsp_hbm, bsp_hbm, wout_hbm, c_hbm, wmod_hbm,
            out_ref,
            x_buf, c_buf, wsp_buf, bsp_buf, k_buf, v_buf, wq_buf, wo_buf, win_buf, wout_buf, wmod_buf,
            q_scr, o_scr, mod_scr, acc_scr, z_scr, sems, *, SK, W):
    HKV = k_buf.shape[0]
    D = wq_buf.shape[0]
    FH = wout_buf.shape[1]
    look = min(LOOKAHEAD, HKV - 1)

    wo_blocks = _blocks(D, 384)
    win_blocks = _blocks(D, 256, 384)
    wout_blocks = _blocks(D, 128, 256, 384)

    S_SMALL, S_WMOD, S_WQ, S_K = 0, 4, 5, 6
    S_V = S_K + HKV
    S_WO = S_V + HKV
    S_WIN = S_WO + len(wo_blocks)
    S_WOUT = S_WIN + len(win_blocks)

    def start_piece(src, dst, rects, sem_id, priority):
        for r0, nr, c0, nc in rects:
            window = (pl.ds(r0, nr), pl.ds(c0, nc))
            pltpu.make_async_copy(src.at[window], dst.at[window], sems.at[sem_id]).start(priority=priority)

    def wait_filled(buf, sem_id):
        pltpu.make_async_copy(buf, buf, sems.at[sem_id]).wait()

    def streams(src, dst, queues, sem_id):
        return tuple([functools.partial(start_piece, src, dst, piece, sem_id, prio) for piece in pieces]
                     for prio, pieces in enumerate(queues))

    k_queues = _two_queues((W, DH), 0, W, K_PHASE)
    v_queues = _two_queues((W, DH), 0, W, V_PHASE)

    def k_stream(g):
        return streams(k_hbm.at[0, g, pl.ds(SK - W, W), :], k_buf.at[g], k_queues, S_K + g)

    def v_stream(g):
        return streams(v_hbm.at[0, g, pl.ds(SK - W, W), :], v_buf.at[g], v_queues, S_V + g)

    def interleave(first, second):
        for i in range(max(len(first), len(second))):
            for starters in (first, second):
                if i < len(starters):
                    starters[i]()

    tail = []
    for src, dst, blocks, sem0, rows in ((wo_hbm, wo_buf, wo_blocks[1:], S_WO + 1, 16),
                                         (win_hbm, win_buf, win_blocks, S_WIN, 32),
                                         (wout_hbm, wout_buf, wout_blocks, S_WOUT, 64)):
        for i, (lo, hi) in enumerate(blocks):
            for r in range(lo, hi, rows):
                rect = (r, min(rows, hi - r), 0, src.shape[1])
                tail.append(functools.partial(start_piece, src, dst, [rect], sem0 + i, 1))

    small = ((c_hbm, c_buf), (x_hbm, x_buf), (wsp_hbm, wsp_buf), (bsp_hbm, bsp_buf))
    for i, (src, dst) in enumerate(small):
        pltpu.make_async_copy(src, dst, sems.at[S_SMALL + i]).start(priority=0)
    weights = [streams(wmod_hbm, wmod_buf, _two_queues(wmod_buf.shape, 0, D), S_WMOD),
               streams(wq_hbm, wq_buf, _two_queues(wq_buf.shape, 0, D), S_WQ),
               streams(wo_hbm, wo_buf, _two_queues(wo_buf.shape, *wo_blocks[0]), S_WO)]
    head0 = [s for chunk in weights for s in chunk[0]]
    head1 = [s for chunk in weights for s in chunk[1]]
    head0 += [s for g in range(look) for stream in (k_stream, v_stream) for s in stream(g)[0]]
    head1 += [s for g in range(look + 1) for stream in (k_stream, v_stream) for s in stream(g)[1]]
    interleave([], head1[:LEAD])
    head1 = head1[LEAD:]
    issued = [0]

    def advance(upto):
        interleave(head0[issued[0]:upto], head1[issued[0]:upto])
        issued[0] = max(issued[0], upto)

    advance(len(weights[0][0]) + 20)
    for i, (_, dst) in enumerate(small):
        wait_filled(dst, S_SMALL + i)
    c = jnp.broadcast_to(c_buf[...].astype(F32), (ROWS, D))
    x = jnp.broadcast_to(x_buf[0].astype(F32), (ROWS, D))
    silu_c = (c * jax.nn.sigmoid(c)).astype(BF16)
    wait_filled(wmod_buf, S_WMOD)
    mod = _dot(silu_c, wmod_buf[...], _NN)
    for i in range(6):
        mod_scr[i] = mod[:, i * D:(i + 1) * D]

    h = (_layernorm(x) * (1.0 + mod_scr[1]) + mod_scr[0]).astype(BF16)
    advance(len(weights[0][0]) + len(weights[1][0]) + 40)
    wait_filled(wq_buf, S_WQ)
    q = _dot(h, wq_buf[...], _NN)
    q = q.astype(BF16).astype(F32) * (DH ** -0.5)
    even = (lax.broadcasted_iota(jnp.int32, (ROWS, DH), 0) % 2) == 0
    for g in range(HKV):
        q_scr[g] = jnp.where(even, q[:, (2 * g) * DH:(2 * g + 1) * DH], q[:, (2 * g + 1) * DH:(2 * g + 2) * DH])
    advance(max(len(head0), len(head1)))

    def kv_head(g, carry, *, steady):
        def enqueue(stream, tail_part):
            if steady:
                interleave(stream(g + look)[0], stream(g + look + 1)[1])
            else:
                @pl.when(g == HKV - look - 1)
                def _():
                    interleave(stream(HKV - 1)[0], tail_part)

        n = len(k_queues[0])
        qg = q_scr[g].astype(BF16)
        enqueue(k_stream, tail[:n])
        wait_filled(k_buf.at[g], S_K + g)
        s = _dot(qg, k_buf[g], _NT)
        e = jnp.exp(s - jnp.max(s, axis=-1, keepdims=True))
        denom = jnp.sum(e, axis=-1, keepdims=True)
        enqueue(v_stream, tail[n:])
        wait_filled(v_buf.at[g], S_V + g)
        o = _dot(e.astype(BF16), v_buf[g], _NN) / denom
        o_scr[g] = jnp.concatenate([jnp.where(even, o, 0.0), jnp.where(even, 0.0, o)], axis=1)
        return carry

    lax.fori_loop(0, HKV - look - 1, functools.partial(kv_head, steady=True), 0)
    lax.fori_loop(HKV - look - 1, HKV, functools.partial(kv_head, steady=False), 0)

    o_all = jnp.concatenate([o_scr[g] for g in range(HKV)], axis=1).astype(BF16)
    for i, (lo, hi) in enumerate(wo_blocks):
        wait_filled(wo_buf.at[pl.ds(lo, hi - lo), :], S_WO + i)
        acc_scr[0, :, lo:hi] = _dot(o_all, wo_buf[lo:hi, :], _NT)
    r = acc_scr[0]
    x1 = x + mod_scr[2] * (r + pltpu.roll(r, 1, 0))

    h2 = (_layernorm(x1) * (1.0 + mod_scr[4]) + mod_scr[3]).astype(BF16)
    for i, (lo, hi) in enumerate(win_blocks):
        wait_filled(win_buf.at[pl.ds(lo, hi - lo), :], S_WIN + i)
        part = _dot(h2[:, lo:hi], win_buf[lo:hi, :], _NN)
        if i == len(win_blocks) - 1:
            z = z_scr[...] + part
        elif i == 0:
            z_scr[...] = part
        else:
            z_scr[...] += part
    z = jax.nn.gelu(z, approximate=True)
    w_sp = wsp_buf[...].astype(F32)
    b_sp = bsp_buf[...].astype(F32).reshape(1, 1)
    gate = w_sp * _layernorm(z[:, FH:]) + b_sp
    zg = (z[:, :FH] * gate).astype(BF16)

    last_lo = wout_blocks[-1][0]
    for i, (lo, hi) in enumerate(wout_blocks):
        wait_filled(wout_buf.at[pl.ds(lo, hi - lo), :], S_WOUT + i)
        y = _dot(zg, wout_buf[lo:hi, :], _NT)
        if lo != last_lo:
            acc_scr[1, :, lo:hi] = y
    x2 = jnp.concatenate([x1[:, :last_lo] + mod_scr[5, :, :last_lo] * acc_scr[1, :, :last_lo],
                          x1[:, last_lo:] + mod_scr[5, :, last_lo:] * y], axis=1)
    out_ref[...] = x2[0:1, :].astype(BF16).reshape(out_ref.shape)


@jax.jit
def pallas_adaLN_cond__sliding_block_cached__mixer_gmlp__decode_kernel(
    A_x: jax.Array,
    A_k_cache: jax.Array,
    A_v_cache: jax.Array,
    A_wq: jax.Array,
    A_wo: jax.Array,
    B_x: jax.Array,
    B_w_in: jax.Array,
    B_w_sp: jax.Array,
    B_b_sp: jax.Array,
    B_w_out: jax.Array,
    c: jax.Array,
    w_mod: jax.Array,
):
    del B_x
    D = A_x.shape[-1]
    HKV, SK = A_k_cache.shape[1], A_k_cache.shape[2]
    W = min(4096, max(256, SK // 4))
    FH = B_w_out.shape[0]
    n_sems = 6 + 2 * HKV + 2 + 3 + 4
    hbm = pl.BlockSpec(memory_space=pltpu.HBM)
    return pl.pallas_call(
        functools.partial(_kernel, SK=SK, W=W),
        out_shape=jax.ShapeDtypeStruct(A_x.shape, BF16),
        in_specs=[hbm] * 11,
        out_specs=pl.BlockSpec(memory_space=pltpu.VMEM),
        scratch_shapes=[
            pltpu.VMEM(A_x.shape, BF16),
            pltpu.VMEM(c.shape, BF16),
            pltpu.VMEM(B_w_sp.shape, BF16),
            pltpu.VMEM(B_b_sp.shape, BF16),
            pltpu.VMEM((HKV, W, DH), BF16),
            pltpu.VMEM((HKV, W, DH), BF16),
            pltpu.VMEM((D, HQ * DH), BF16),
            pltpu.VMEM((D, HQ * DH), BF16),
            pltpu.VMEM((D, 2 * FH), BF16),
            pltpu.VMEM((D, FH), BF16),
            pltpu.VMEM((D, 6 * D), BF16),
            pltpu.VMEM((HKV, ROWS, DH), F32),
            pltpu.VMEM((HKV, ROWS, 2 * DH), F32),
            pltpu.VMEM((6, ROWS, D), F32),
            pltpu.VMEM((2, ROWS, D), F32),
            pltpu.VMEM((ROWS, 2 * FH), F32),
            pltpu.SemaphoreType.DMA((n_sems,)),
        ],
        compiler_params=pltpu.CompilerParams(
            vmem_limit_bytes=100 * 1024 * 1024,
            disable_semaphore_checks=True,
        ),
    )(A_x, A_k_cache, A_v_cache, A_wq, A_wo.T, B_w_in, B_w_sp, B_b_sp, B_w_out.T, c, w_mod)
```

```python
import functools

import jax
import jax.numpy as jnp
from jax import lax
import jax.experimental.pallas as pl
import jax.experimental.pallas.tpu as pltpu

HQ, DH = 16, 256
EPS = 1e-5
BF16 = jnp.bfloat16
F32 = jnp.float32
ROWS = 8

TILE_R, TILE_C = 8, 128
KV_CYCLE = (30, 34)
K_PHASE, V_PHASE = 16, 24
W_CYCLE = (48, 16)
WMOD_CYCLE = (63, 21)
LEAD = 32
LOOKAHEAD = 2

_NN = (((1,), (0,)), ((), ()))
_NT = (((1,), (1,)), ((), ()))


def _dot(a, b, dims):
    return lax.dot_general(a, b, dims, preferred_element_type=F32)


def _layernorm(x):
    m = jnp.mean(x, axis=-1, keepdims=True)
    xc = x - m
    v = jnp.mean(xc * xc, axis=-1, keepdims=True)
    return xc * lax.rsqrt(v + EPS)


def _blocks(total, *cuts):
    edges = [0] + [c for c in cuts if 0 < c < total] + [total]
    return list(zip(edges[:-1], edges[1:]))


def _rects(t0, t1, col_tiles):
    out = []
    while t0 < t1:
        r, c = divmod(t0, col_tiles)
        if c == 0 and t1 - t0 >= col_tiles:
            n = (t1 - t0) // col_tiles
            out.append((r * TILE_R, n * TILE_R, 0, col_tiles * TILE_C))
            t0 += n * col_tiles
        else:
            n = min(col_tiles - c, t1 - t0)
            out.append((r * TILE_R, TILE_R, c * TILE_C, n * TILE_C))
            t0 += n
    return out


def _two_queues(shape, lo, hi, cycle, phase=0):
    col_tiles = shape[1] // TILE_C
    t, end = lo // TILE_R * col_tiles, hi // TILE_R * col_tiles
    queues, held = ([], []), []
    pos = (t + phase) % sum(cycle)
    while t < end:
        prio = 0 if pos < cycle[0] else 1
        n = min((cycle[0] if prio == 0 else sum(cycle)) - pos, end - t)
        piece = _rects(t, t + n, col_tiles)
        if prio == 0 and not queues[1] and n < cycle[0] and not held:
            held = piece
        else:
            queues[prio].append(held + piece if prio == 0 else piece)
            held = [] if prio == 0 else held
        t, pos = t + n, (pos + n) % sum(cycle)
    if held:
        queues[0].append(held)
    return queues


def _kernel(x_hbm, k_hbm, v_hbm, wq_hbm, wo_hbm, win_hbm, wsp_hbm, bsp_hbm, wout_hbm, c_hbm, wmod_hbm,
            out_ref,
            x_buf, c_buf, wsp_buf, bsp_buf, k_buf, v_buf, wq_buf, wo_buf, win_buf, wout_buf, wmod_buf,
            q_scr, o_scr, mod_scr, acc_scr, z_scr, sems, *, SK, W):
    HKV = k_buf.shape[0]
    D = wq_buf.shape[0]
    FH = wout_buf.shape[1]
    look = min(LOOKAHEAD, HKV - 1)

    wo_blocks = _blocks(D, 384)
    win_blocks = _blocks(D, 256, 384)
    wout_blocks = _blocks(D, 128, 256, 384)

    S_SMALL, S_WMOD, S_WQ, S_K = 0, 4, 5, 6
    S_V = S_K + HKV
    S_WO = S_V + HKV
    S_WIN = S_WO + len(wo_blocks)
    S_WOUT = S_WIN + len(win_blocks)

    def start_piece(src, dst, rects, sem_id, priority):
        for r0, nr, c0, nc in rects:
            window = (pl.ds(r0, nr), pl.ds(c0, nc))
            pltpu.make_async_copy(src.at[window], dst.at[window], sems.at[sem_id]).start(priority=priority)

    def wait_filled(buf, sem_id):
        pltpu.make_async_copy(buf, buf, sems.at[sem_id]).wait()

    def streams(src, dst, queues, sem_id):
        return tuple([functools.partial(start_piece, src, dst, piece, sem_id, prio) for piece in pieces]
                     for prio, pieces in enumerate(queues))

    k_queues = _two_queues((W, DH), 0, W, KV_CYCLE, K_PHASE)
    v_queues = _two_queues((W, DH), 0, W, KV_CYCLE, V_PHASE)

    def k_stream(g):
        return streams(k_hbm.at[0, g, pl.ds(SK - W, W), :], k_buf.at[g], k_queues, S_K + g)

    def v_stream(g):
        return streams(v_hbm.at[0, g, pl.ds(SK - W, W), :], v_buf.at[g], v_queues, S_V + g)

    def interleave(first, second):
        for i in range(max(len(first), len(second))):
            for starters in (first, second):
                if i < len(starters):
                    starters[i]()

    tail = []
    for src, dst, blocks, sem0, rows in ((wo_hbm, wo_buf, wo_blocks[1:], S_WO + 1, 16),
                                         (win_hbm, win_buf, win_blocks, S_WIN, 32),
                                         (wout_hbm, wout_buf, wout_blocks, S_WOUT, 64)):
        for i, (lo, hi) in enumerate(blocks):
            for r in range(lo, hi, rows):
                rect = (r, min(rows, hi - r), 0, src.shape[1])
                tail.append(functools.partial(start_piece, src, dst, [rect], sem0 + i, 1))

    small = ((c_hbm, c_buf), (x_hbm, x_buf), (wsp_hbm, wsp_buf), (bsp_hbm, bsp_buf))
    for i, (src, dst) in enumerate(small):
        pltpu.make_async_copy(src, dst, sems.at[S_SMALL + i]).start(priority=0)
    weights = [streams(wmod_hbm, wmod_buf, _two_queues(wmod_buf.shape, 0, D, WMOD_CYCLE), S_WMOD),
               streams(wq_hbm, wq_buf, _two_queues(wq_buf.shape, 0, D, W_CYCLE), S_WQ),
               streams(wo_hbm, wo_buf, _two_queues(wo_buf.shape, *wo_blocks[0], W_CYCLE), S_WO)]
    head0 = [s for chunk in weights for s in chunk[0]]
    head1 = [s for chunk in weights for s in chunk[1]]
    head0 += [s for g in range(look) for stream in (k_stream, v_stream) for s in stream(g)[0]]
    head1 += [s for g in range(look + 1) for stream in (k_stream, v_stream) for s in stream(g)[1]]
    interleave([], head1[:LEAD])
    head1 = head1[LEAD:]
    issued = [0]

    def advance(upto):
        interleave(head0[issued[0]:upto], head1[issued[0]:upto])
        issued[0] = max(issued[0], upto)

    advance(len(weights[0][0]) + 20)
    for i, (_, dst) in enumerate(small):
        wait_filled(dst, S_SMALL + i)
    c = jnp.broadcast_to(c_buf[...].astype(F32), (ROWS, D))
    x = jnp.broadcast_to(x_buf[0].astype(F32), (ROWS, D))
    silu_c = (c * jax.nn.sigmoid(c)).astype(BF16)
    wait_filled(wmod_buf, S_WMOD)
    mod = _dot(silu_c, wmod_buf[...], _NN)
    for i in range(6):
        mod_scr[i] = mod[:, i * D:(i + 1) * D]

    h = (_layernorm(x) * (1.0 + mod_scr[1]) + mod_scr[0]).astype(BF16)
    advance(len(weights[0][0]) + len(weights[1][0]) + 40)
    wait_filled(wq_buf, S_WQ)
    q = _dot(h, wq_buf[...], _NN)
    q = q.astype(BF16).astype(F32) * (DH ** -0.5)
    even = (lax.broadcasted_iota(jnp.int32, (ROWS, DH), 0) % 2) == 0
    for g in range(HKV):
        q_scr[g] = jnp.where(even, q[:, (2 * g) * DH:(2 * g + 1) * DH], q[:, (2 * g + 1) * DH:(2 * g + 2) * DH])
    advance(max(len(head0), len(head1)))

    def kv_head(g, carry, *, steady):
        def enqueue(stream, tail_part):
            if steady:
                interleave(stream(g + look)[0], stream(g + look + 1)[1])
            else:
                @pl.when(g == HKV - look - 1)
                def _():
                    interleave(stream(HKV - 1)[0], tail_part)

        n = len(k_queues[0])
        qg = q_scr[g].astype(BF16)
        enqueue(k_stream, tail[:n])
        wait_filled(k_buf.at[g], S_K + g)
        s = _dot(qg, k_buf[g], _NT)
        e = jnp.exp(s - jnp.max(s, axis=-1, keepdims=True))
        denom = jnp.sum(e, axis=-1, keepdims=True)
        enqueue(v_stream, tail[n:])
        wait_filled(v_buf.at[g], S_V + g)
        o = _dot(e.astype(BF16), v_buf[g], _NN) / denom
        o_scr[g] = jnp.concatenate([jnp.where(even, o, 0.0), jnp.where(even, 0.0, o)], axis=1)
        return carry

    lax.fori_loop(0, HKV - look - 1, functools.partial(kv_head, steady=True), 0)
    lax.fori_loop(HKV - look - 1, HKV, functools.partial(kv_head, steady=False), 0)

    o_all = jnp.concatenate([o_scr[g] for g in range(HKV)], axis=1).astype(BF16)
    for i, (lo, hi) in enumerate(wo_blocks):
        wait_filled(wo_buf.at[pl.ds(lo, hi - lo), :], S_WO + i)
        acc_scr[0, :, lo:hi] = _dot(o_all, wo_buf[lo:hi, :], _NT)
    r = acc_scr[0]
    x1 = x + mod_scr[2] * (r + pltpu.roll(r, 1, 0))

    h2 = (_layernorm(x1) * (1.0 + mod_scr[4]) + mod_scr[3]).astype(BF16)
    for i, (lo, hi) in enumerate(win_blocks):
        wait_filled(win_buf.at[pl.ds(lo, hi - lo), :], S_WIN + i)
        part = _dot(h2[:, lo:hi], win_buf[lo:hi, :], _NN)
        if i == len(win_blocks) - 1:
            z = z_scr[...] + part
        elif i == 0:
            z_scr[...] = part
        else:
            z_scr[...] += part
    z = jax.nn.gelu(z, approximate=True)
    w_sp = wsp_buf[...].astype(F32)
    b_sp = bsp_buf[...].astype(F32).reshape(1, 1)
    gate = w_sp * _layernorm(z[:, FH:]) + b_sp
    zg = (z[:, :FH] * gate).astype(BF16)

    last_lo = wout_blocks[-1][0]
    for i, (lo, hi) in enumerate(wout_blocks):
        wait_filled(wout_buf.at[pl.ds(lo, hi - lo), :], S_WOUT + i)
        y = _dot(zg, wout_buf[lo:hi, :], _NT)
        if lo != last_lo:
            acc_scr[1, :, lo:hi] = y
    x2 = jnp.concatenate([x1[:, :last_lo] + mod_scr[5, :, :last_lo] * acc_scr[1, :, :last_lo],
                          x1[:, last_lo:] + mod_scr[5, :, last_lo:] * y], axis=1)
    out_ref[...] = x2[0:1, :].astype(BF16).reshape(out_ref.shape)


@jax.jit
def pallas_adaLN_cond__sliding_block_cached__mixer_gmlp__decode_kernel(
    A_x: jax.Array,
    A_k_cache: jax.Array,
    A_v_cache: jax.Array,
    A_wq: jax.Array,
    A_wo: jax.Array,
    B_x: jax.Array,
    B_w_in: jax.Array,
    B_w_sp: jax.Array,
    B_b_sp: jax.Array,
    B_w_out: jax.Array,
    c: jax.Array,
    w_mod: jax.Array,
):
    del B_x
    D = A_x.shape[-1]
    HKV, SK = A_k_cache.shape[1], A_k_cache.shape[2]
    W = min(4096, max(256, SK // 4))
    FH = B_w_out.shape[0]
    n_sems = 6 + 2 * HKV + 2 + 3 + 4
    hbm = pl.BlockSpec(memory_space=pltpu.HBM)
    return pl.pallas_call(
        functools.partial(_kernel, SK=SK, W=W),
        out_shape=jax.ShapeDtypeStruct(A_x.shape, BF16),
        in_specs=[hbm] * 11,
        out_specs=pl.BlockSpec(memory_space=pltpu.VMEM),
        scratch_shapes=[
            pltpu.VMEM(A_x.shape, BF16),
            pltpu.VMEM(c.shape, BF16),
            pltpu.VMEM(B_w_sp.shape, BF16),
            pltpu.VMEM(B_b_sp.shape, BF16),
            pltpu.VMEM((HKV, W, DH), BF16),
            pltpu.VMEM((HKV, W, DH), BF16),
            pltpu.VMEM((D, HQ * DH), BF16),
            pltpu.VMEM((D, HQ * DH), BF16),
            pltpu.VMEM((D, 2 * FH), BF16),
            pltpu.VMEM((D, FH), BF16),
            pltpu.VMEM((D, 6 * D), BF16),
            pltpu.VMEM((HKV, ROWS, DH), F32),
            pltpu.VMEM((HKV, ROWS, 2 * DH), F32),
            pltpu.VMEM((6, ROWS, D), F32),
            pltpu.VMEM((2, ROWS, D), F32),
            pltpu.VMEM((ROWS, 2 * FH), F32),
            pltpu.SemaphoreType.DMA((n_sems,)),
        ],
        compiler_params=pltpu.CompilerParams(
            vmem_limit_bytes=100 * 1024 * 1024,
            disable_semaphore_checks=True,
        ),
    )(A_x, A_k_cache, A_v_cache, A_wq, A_wo.T, B_w_in, B_w_sp, B_b_sp, B_w_out.T, c, w_mod)
```
